```python
import os as _os
_os.environ.setdefault("JAX_PLATFORMS", "cpu")
import jax
import jax.numpy as jnp

def _softmax(x, axis=-1):
    return jax.nn.softmax(x, axis=axis)
def _gelu(x):
    return jax.nn.gelu(x, approximate=True)
def _silu(x):
    return jax.nn.silu(x)
def _sigmoid(x):
    return jax.nn.sigmoid(x)
def _layernorm(x, axis=-1, eps=1e-5):
    m = jnp.mean(x, axis=axis, keepdims=True)
    v = jnp.var(x, axis=axis, keepdims=True)
    return (x - m) / jnp.sqrt(v + eps)
def _scatter_add(tgt, idx, src, axis=0):
    return tgt.at[idx].add(src)
def _segment_sum(src, seg, n):
    return jax.ops.segment_sum(src, seg, n)
class _Rng:
    def __init__(self, key):
        self._k = key
    def _next(self):
        self._k, sub = jax.random.split(self._k)
        return sub
    def normal(self, shape):
        return jax.random.normal(self._next(), shape, dtype=jnp.bfloat16)
    def randint(self, lo, hi, shape):
        return jax.random.randint(self._next(), shape, lo, hi, dtype=jnp.int32)
    def uniform(self, shape, lo=0.0, hi=1.0):
        return jax.random.uniform(self._next(), shape, jnp.bfloat16, lo, hi)
    def permutation(self, n):
        return jax.random.permutation(self._next(), n)


kernel_name = 'concat_heads__grouped_kv_mqa__sliding_block__prompt'

def setup_inputs():
    _rng = _Rng(jax.random.key(int.from_bytes(__import__("os").urandom(4), "little")))
    _w = (lambda a: (lambda t: t.astype(jnp.bfloat16) if jnp.issubdtype(t.dtype, jnp.floating) else t)(jnp.asarray(a)))
    def _A_setup():
        B, S, D, H = 1, 2048, 576, 32
        Dh = D // H
        return {
            "x": _w((lambda *s: _rng.normal(s) * 0.05)(B, S, D)),
            "wq": _w((lambda *s: _rng.normal(s) * 1.6)(D, H * Dh)),
            "wk": _w((lambda *s: _rng.normal(s) * 1.6)(D, Dh)),
            "wv": _w((lambda *s: _rng.normal(s) * 0.1)(D, Dh)),
            "wo": _w((lambda *s: _rng.normal(s) * 0.1)(H * Dh, D)),
        }
    _A_in = _A_setup()

    def _B_setup():
        B, S, D = 1, 2048, 576
        return {
            "x": _w((lambda *s: _rng.normal(s) * 0.2)(B, S, D)),
            "wqkv": _w((lambda *s: _rng.normal(s) * 0.2)(D, 3 * D)),
            "wo": _w((lambda *s: _rng.normal(s) * 0.05)(D, D)),
        }
    _B_in = _B_setup()

    return {
        "A_x": _A_in["x"],
        "A_wq": _A_in["wq"],
        "A_wk": _A_in["wk"],
        "A_wv": _A_in["wv"],
        "A_wo": _A_in["wo"],
        "B_x": _B_in["x"],
        "B_wqkv": _B_in["wqkv"],
        "B_wo": _B_in["wo"],
    }

def reference(A_x, A_wq, A_wk, A_wv, A_wo, B_x, B_wqkv, B_wo):
    def _A_ref(x, wq, wk, wv, wo):
        B, S, D = x.shape
        H = 32
        Dh = D // H
        q = (lambda x, *d: x.transpose(*d))((x @ wq).reshape(B, S, H, Dh), 0, 2, 1, 3)
        k = x @ wk
        v = x @ wv
        scores = jnp.einsum("bhqd,bkd->bhqk", q, k) * (Dh ** -0.5)
        p = _softmax(scores, axis=-1)
        o = jnp.einsum("bhqk,bkd->bhqd", p, v)
        return (lambda x, *d: x.transpose(*d))(o, 0, 2, 1, 3).reshape(B, S, H * Dh) @ wo

    def _B_ref(x, wqkv, wo):
        B, S, D = x.shape
        H = 32; Dh = D // H; W = 256
        qkv = (lambda x, *d: x.transpose(*d))((x @ wqkv).reshape(B, S, 3, H, Dh), 2, 0, 3, 1, 4)
        q, k, v = qkv[0], qkv[1], qkv[2]
        scores = jnp.einsum("bhqd,bhkd->bhqk", q, k) * (Dh ** -0.5)
        idx = jnp.arange(S)
        mask = (idx[:, None] - idx[None, :] >= 0) & (idx[:, None] - idx[None, :] < W)
        scores = jnp.where(mask[None, None], scores, -1e9)
        p = _softmax(scores, axis=-1)
        o = jnp.einsum("bhqk,bhkd->bhqd", p, v)
        return (lambda x, *d: x.transpose(*d))(o, 0, 2, 1, 3).reshape(B, S, D) @ wo

    a = _A_ref(A_x, A_wq, A_wk, A_wv, A_wo)
    b = _B_ref(B_x, B_wqkv, B_wo)
    return jnp.concatenate([a, b], axis=-1)
```

```python
import math

import jax
import jax.numpy as jnp
from jax import lax
import jax.experimental.pallas as pl
import jax.experimental.pallas.tpu as pltpu

S = 2048
D = 576
H = 32
DH = D // H
W = 256
F32 = jnp.float32
BF16 = jnp.bfloat16
QSCALE = (DH ** -0.5) * math.log2(math.e)
NEG = -1e9 * math.log2(math.e)

QB = 512
KC = 128
PB = 512
GH = 4
GROWS = 80

_NN = (((1,), (0,)), ((), ()))


def _mm(a, b):
    return lax.dot_general(a, b, _NN, preferred_element_type=F32)


def _kernel(xa_hbm, wq_hbm, wk_hbm, wv_hbm, woa_hbm, xb_hbm, wqkv_hbm, wob_hbm,
            out_hbm,
            xa, wq, wk, wv, woa, xb, wqkv, wob,
            wat, wbt, woat, wobt,
            qa, ka, va, sa, oa,
            qb, kb, vb, ob,
            obuf, in_sem, x_sem, out_sem):
    nb = S // PB

    def x_copy(src, dst, base, c):
        cols = pl.ds(c * PB, PB)
        return pltpu.make_async_copy(src.at[:, cols], dst.at[:, cols], x_sem.at[base + c])

    w_copies = [pltpu.make_async_copy(src, dst, in_sem.at[i]) for i, (src, dst) in enumerate(
        [(wq_hbm, wq), (wk_hbm, wk), (wv_hbm, wv),
         (wqkv_hbm, wqkv), (woa_hbm, woa), (wob_hbm, wob)])]

    for cp in w_copies[:3]:
        cp.start()
    for c in range(nb):
        x_copy(xa_hbm, xa, 0, c).start()
    w_copies[3].start()
    for c in range(nb):
        x_copy(xb_hbm, xb, nb, c).start()
    w_copies[4].start()
    w_copies[5].start()

    oa[...] = jnp.zeros(oa.shape, F32)
    ob[...] = jnp.zeros(ob.shape, F32)
    kb[:, 0:W, :] = jnp.zeros((H // GH, W, GROWS), BF16)
    vb[:, 0:W] = jnp.zeros((D, W), F32)

    for cp in w_copies[:3]:
        cp.wait()
    wat[0:D, :] = wq[...].T
    pad = jnp.zeros((32 - DH, D), F32)
    wat[D:D + 32, :] = jnp.concatenate([wk[...].astype(F32), pad], axis=0).astype(BF16)
    wat[D + 32:D + 64, :] = jnp.concatenate([wv[...].astype(F32), pad], axis=0).astype(BF16)

    row24 = lax.broadcasted_iota(jnp.int32, (24, PB), 0)

    def proj_a(c, _):
        x_copy(xa_hbm, xa, 0, c).wait()
        cols = pl.ds(pl.multiple_of(c * PB, PB), PB)
        r = _mm(wat[...], xa[:, cols])
        qa[:, cols] = (r[0:D] * QSCALE).astype(BF16)
        kt = r[D:D + 32]
        for j in range(8):
            kj = kt if j == 0 else pltpu.roll(kt, 2 * j, 0)
            ka[j, cols, :] = kj.T.astype(BF16)
        vt = r[D + 32:D + 56].astype(BF16).astype(F32)
        for j in range(4):
            vj = vt if j == 0 else pltpu.roll(vt, 2 * j, 0)
            head = (row24 >= 2 * j) & (row24 < 2 * j + DH)
            va[j, :, cols] = jnp.where(head, vj, 1.0)
        return 0

    lax.fori_loop(0, nb, proj_a, 0)

    def a_scores(i):
        h = i % H
        cols = pl.ds(pl.multiple_of((i // H) * QB, QB), QB)
        start = pl.multiple_of(((h * DH) // 16) * 16, 16)
        q = qa[pl.ds(start, 32), cols]
        kh = ka.at[(h * DH - start) // 2]

        def f(c, m):
            rows = pl.ds(c * KC, KC)
            s = _mm(kh[rows, :], q)
            sa[rows, :] = s
            mc = jnp.max(s.reshape(KC // 8, 8, QB), axis=0)
            return mc if m is None else jnp.maximum(m, mc)
        return f

    def a_values(i, m):
        h = i % H
        cols = pl.ds(pl.multiple_of((i // H) * QB, QB), QB)
        start = pl.multiple_of(((h * DH) // 8) * 8, 8)
        off = h * DH - start
        vh = va.at[off // 2]

        def f(c, acc):
            rows = pl.ds(c * KC, KC)
            p = jnp.exp2(sa[rows, :] - m).astype(BF16)
            a = _mm(vh[:, rows], p)
            return a if acc is None else acc + a

        def done(acc):
            den = jnp.where(off == 0, acc[23:24], acc[0:1])
            o = acc * (1.0 / den)
            first = pl.ds(start, 8)
            row8 = lax.broadcasted_iota(jnp.int32, (8, QB), 0)
            oa[first, cols] = jnp.where(row8 >= off, o[0:8], oa[first, cols])
            oa[pl.ds(start + 8, 16), cols] = o[8:24]
        return f, done

    nsteps = (S // QB) * H
    nchunk = S // KC

    scores = a_scores(0)
    m = None
    for c in range(nchunk):
        m = scores(c, m)

    def a_step(i, m_prev):
        values, done = a_values(i - 1, m_prev)
        scores = a_scores(i)
        m, acc = None, None
        for c in range(nchunk):
            acc = values(c, acc)
            m = scores(c, m)
        done(acc)
        return jnp.max(m, axis=0, keepdims=True)

    m = lax.fori_loop(1, nsteps, a_step, jnp.max(m, axis=0, keepdims=True))
    values, done = a_values(nsteps - 1, m)
    acc = None
    for c in range(nchunk):
        acc = values(c, acc)
    done(acc)

    w_copies[3].wait()
    wbt[...] = wqkv[...].T

    def proj_b(c, _):
        x_copy(xb_hbm, xb, nb, c).wait()
        cols = pl.ds(pl.multiple_of(c * PB, PB), PB)
        pcols = pl.ds(pl.multiple_of(c * PB + W, W), PB)
        x = xb[:, cols]
        qb[:, cols] = (_mm(wbt[0:D, :], x) * QSCALE).astype(BF16)
        kt = _mm(wbt[D:2 * D, :], x).astype(BF16)
        for g in range(H // GH):
            start = (g * GH * DH) // 16 * 16
            kb[g, pcols, :] = kt[start:start + GROWS].T
        vb[:, pcols] = _mm(wbt[2 * D:3 * D, :], x).astype(BF16).astype(F32)
        return 0

    lax.fori_loop(0, nb, proj_b, 0)

    r_i = lax.broadcasted_iota(jnp.int32, (128, 128), 0)
    c_i = lax.broadcasted_iota(jnp.int32, (128, 128), 1)
    grow = lax.broadcasted_iota(jnp.int32, (GROWS, 128), 0)
    row24b = lax.broadcasted_iota(jnp.int32, (24, 3 * 128), 0)
    row24o = lax.broadcasted_iota(jnp.int32, (24, 128), 0)

    def b_step(j, _):
        cols = pl.ds(pl.multiple_of(j * 128, 128), 128)
        keys = pl.ds(pl.multiple_of(j * 128, 128), 3 * 128)
        upper = r_i > c_i
        keep0 = upper & (j >= 2)
        keep1 = jnp.broadcast_to(j >= 1, (128, 128))

        def scores(g):
            start = (g * GH * DH) // 16 * 16
            q = qb[start:start + GROWS, cols].astype(F32)
            qs = []
            for t in range(GH):
                lo = (g * GH + t) * DH - start
                qs.append(jnp.where((grow >= lo) & (grow < lo + DH), q, 0.0).astype(BF16))
            return _mm(kb[g, keys, :], jnp.concatenate(qs, axis=1))

        def values(g, s):
            outs = []
            for t in range(GH):
                h = g * GH + t
                st = s[:, t * 128:(t + 1) * 128]
                s02 = jnp.where(upper, jnp.where(keep0, st[0:128], NEG), st[256:384])
                s1 = jnp.where(keep1, st[128:256], NEG)
                m = jnp.max(jnp.maximum(s02, s1), axis=0, keepdims=True)
                e02 = jnp.exp2(s02 - m)
                p = jnp.concatenate([jnp.where(upper, e02, 0.0), jnp.exp2(s1 - m),
                                     jnp.where(upper, 0.0, e02)], axis=0).astype(BF16)
                start = (h * DH) // 8 * 8
                off = h * DH - start
                v = jnp.where((row24b >= off) & (row24b < off + DH), vb[start:start + 24, keys], 1.0)
                acc = _mm(v, p)
                den = acc[23:24] if off == 0 else acc[0:1]
                outs.append(acc * (1.0 / den))
            rows = [outs[0][0:16]]
            for t in range(1, GH):
                keep = row24o[0:8] >= 2 * t
                rows.append(jnp.where(keep, outs[t][0:8], outs[t - 1][16:24]))
                rows.append(outs[t][8:16])
            rows.append(outs[GH - 1][16:24])
            ob[g * GH * DH:(g + 1) * GH * DH, cols] = jnp.concatenate(rows, axis=0)

        s = scores(0)
        for g in range(H // GH):
            s_next = scores(g + 1) if g + 1 < H // GH else None
            values(g, s)
            s = s_next
        return 0

    lax.fori_loop(0, S // 128, b_step, 0)

    w_copies[4].wait()
    w_copies[5].wait()
    woat[...] = woa[...].T
    wobt[...] = wob[...].T

    def out_copy(c):
        rows = pl.ds(c * PB, PB)
        return pltpu.make_async_copy(obuf.at[rows, :], out_hbm.at[rows, :], out_sem.at[c])

    def proj_o(c, _):
        cols = pl.ds(pl.multiple_of(c * PB, PB), PB)
        ya = _mm(woat[...], oa[:, cols].astype(BF16)).astype(BF16)
        yb = _mm(wobt[...], ob[:, cols].astype(BF16)).astype(BF16)
        obuf[cols, :] = jnp.concatenate([ya, yb], axis=0).T
        out_copy(c).start()
        return 0

    lax.fori_loop(0, nb, proj_o, 0)
    for c in range(nb):
        out_copy(c).wait()


@jax.jit
def pallas_concat_heads__grouped_kv_mqa__sliding_block__prompt_kernel(
    A_x: jax.Array,
    A_wq: jax.Array,
    A_wk: jax.Array,
    A_wv: jax.Array,
    A_wo: jax.Array,
    B_x: jax.Array,
    B_wqkv: jax.Array,
    B_wo: jax.Array,
):
    hbm = pl.BlockSpec(memory_space=pltpu.HBM)
    vmem = pltpu.VMEM
    nb = S // PB
    out = pl.pallas_call(
        _kernel,
        in_specs=[hbm] * 8,
        out_specs=hbm,
        out_shape=jax.ShapeDtypeStruct((S, 2 * D), BF16),
        scratch_shapes=[
            vmem((D, S), BF16), vmem((D, D), BF16), vmem((DH, D), BF16), vmem((DH, D), BF16),
            vmem((D, D), BF16), vmem((D, S), BF16), vmem((D, 3 * D), BF16), vmem((D, D), BF16),
            vmem((D + 64, D), BF16), vmem((3 * D, D), BF16), vmem((D, D), BF16), vmem((D, D), BF16),
            vmem((D, S), BF16), vmem((8, S, 32), BF16), vmem((4, 24, S), F32),
            vmem((S, QB), F32), vmem((D, S), F32),
            vmem((D, S), BF16), vmem((H // GH, S + W, GROWS), BF16), vmem((D, S + W), F32),
            vmem((D, S), F32),
            vmem((S, 2 * D), BF16),
            pltpu.SemaphoreType.DMA((6,)), pltpu.SemaphoreType.DMA((2 * nb,)),
            pltpu.SemaphoreType.DMA((nb,)),
        ],
        compiler_params=pltpu.CompilerParams(vmem_limit_bytes=100 * 1024 * 1024),
        name="mqa_swa_fused",
    )(A_x[0].T, A_wq, A_wk.T, A_wv.T, A_wo, B_x[0].T, B_wqkv, B_wo)
    return out[None]
```

```python
import math

import jax
import jax.numpy as jnp
from jax import lax
import jax.experimental.pallas as pl
import jax.experimental.pallas.tpu as pltpu

S = 2048
D = 576
H = 32
DH = D // H
W = 256
F32 = jnp.float32
BF16 = jnp.bfloat16
U32 = jnp.uint32
LOG2E = math.log2(math.e)
QSCALE = (DH ** -0.5) * LOG2E
NEG = -1e9 * LOG2E

QB = 512
NB = S // QB
NT = QB // 128
KC = 128
NC = S // KC
GH = 4
NG = H // GH
GR = GH * DH
GP = 80
BAND = 32
BR = W + BAND
DM = D // 128 * 128

NS = 17
NSC = 12
NS0 = 0
LINKS = 16.4
PD = 12
GQ = 0
DUP = 4
AU = 1
TOFF = 1
TGAP = 3
TPAD = 2
SLOTS = [(NS * (c - NS0 + 1)) // (NSC - NS0) - (NS * (c - NS0)) // (NSC - NS0) if NS0 <= c < NSC else 0
         for c in range(NC)]
SLOT_KEY = [(c + 1) * KC - 16 * (SLOTS[c] - x) for c in range(NC) for x in range(SLOTS[c])]
_tslot = lambda x, d: x * (DH + TGAP) + d + TOFF
TROWS = 2 * DH + TGAP + TOFF + TPAD

M_QUERY, M_OLD, M_NEW, M_KEY, M_ROWS = 0, 160, 224, 288, 320


def _mm(a, b):
    return lax.dot_general(a, b, (((1,), (0,)), ((), ())), preferred_element_type=F32)


def _pack(x):
    return pltpu.bitcast(x.astype(BF16), U32)


def _bf16(x):
    return pltpu.bitcast(x, BF16)


def _iota(shape, dim):
    return lax.broadcasted_iota(jnp.int32, shape, dim)


def _tile(i):
    return pl.ds(pl.multiple_of(i * 128, 128), 128)


def _always(step):
    return _iota((8, 128), 0) <= step + 8


class _VpuScores:
    def __init__(self, step):
        self.always, self.count, self.prev, self.last = _always(step), 0, None, None

    def __call__(self, keys, query):
        n = self.count
        release = min(int((n + 1) * LINKS) - int(n * LINKS) - 1 - (GQ > 0), DH - 1)
        acc, prev = [None, None], self.prev
        for d in range(DH):
            q = query(d)
            if GQ and d == 0 and prev is not None:
                q = jnp.where(self.always, q, prev[GQ - 1])
            for x in range(2):
                pr = keys(x, d) * q
                if not GQ and d == 0 and prev is not None:
                    pr = jnp.where(self.always, pr, prev[x])
                if d == PD and x == 0 and self.last is not None:
                    pr = jnp.where(self.always, pr, self.last)
                acc[x] = pr if d == 0 else acc[x] + pr
            if d == release:
                self.prev = list(acc)
        e = pltpu.pack_elementwise([jnp.exp2(acc[0]), jnp.exp2(acc[1])], packed_dtype=BF16)
        self.count, self.last = n + 1, pltpu.bitcast(e, F32)
        return e


def _normalise(acc, u, z):
    den = acc[23:24] if u == 0 else acc[0:1]
    r = pltpu.reciprocal(den, approx=True)
    r = r * (2.0 - den * r)
    big = r * (2.0 ** 20)
    sq = acc * acc
    return acc * r, z + (sq[0:8] + sq[8:16] + sq[16:24] + big * big)


def _stitch(outs):
    row = _iota((8, 128), 0)
    rows = [outs[0][0:16]]
    for h in range(1, GH):
        rows.append(jnp.where(row >= 2 * h, outs[h][0:8], outs[h - 1][16:24]))
        rows.append(outs[h][8:16])
    rows.append(outs[GH - 1][16:24])
    return jnp.concatenate(rows, axis=0)


def _kernel(xa_hbm, wq_hbm, wk_hbm, wv_hbm, woa_hbm, xb_hbm, wqkv_hbm, wob_hbm,
            out_hbm,
            xa, wsq, wk, wv, xb, wqkv,
            wat, wbt, wot, tail,
            qa, qs, ka, kf, va, ktab, pa, oa,
            qb, kb, vb, eb, ob, msk,
            ybuf, obuf, in_sem, x_sem, out_sem):

    def x_copy(c):
        cols = pl.ds(c * QB, QB)
        return pltpu.make_async_copy(xa_hbm.at[:, cols], xa.at[:, cols], x_sem.at[c])

    wq_copy, wk_copy, wv_copy, wqkv_copy, xb_copy, woa_copy, wob_copy = [
        pltpu.make_async_copy(src, dst, in_sem.at[i]) for i, (src, dst) in enumerate(
            [(wq_hbm, wsq.at[0]), (wk_hbm, wk), (wv_hbm, wv), (wqkv_hbm, wqkv), (xb_hbm, xb),
             (woa_hbm, wsq.at[1]), (wob_hbm, wsq.at[2])])]

    for cp in (wq_copy, wk_copy, wv_copy, x_copy(0)):
        cp.start()

    ones = jnp.uint32(0x3F803F80)
    pa[S // 2:, :] = jnp.full((S // 2, QB), ones, U32)
    eb[BR // 2:, :] = jnp.full((BR // 2, QB), ones, U32)
    vb[GH:, :, S - 384:] = jnp.ones((GH, 24, 384), F32)
    ybuf[...] = jnp.full(ybuf.shape, ones, U32)

    n, full, none = BAND // 2, jnp.uint32(0xFFFFFFFF), jnp.uint32(0)
    for t in range(GH):
        head = ((_iota((GP // 2, 128), 1) >> 5) + t) & (GH - 1)
        row = _iota((GP // 2, 128), 0)
        msk[pl.ds(M_QUERY + t * (GP // 2), GP // 2), :] = jnp.where(
            (row >= head * (DH // 2)) & (row < (head + 1) * (DH // 2)), full, none)
        lane_head = sum(jnp.where(_iota((8, 128), 1) >= x * DH, 1, 0) for x in range(1, GH))
        msk[pl.ds(M_KEY + 8 * t, 8), :] = ((lane_head + (GH - t)) & (GH - 1)).astype(U32)
    lane = _iota((n, 128), 1)
    band, pos, key = lane >> 5, lane & (BAND - 1), 2 * _iota((n, 128), 0)
    newer = (jnp.where(key > pos, jnp.uint32(0xFFFF), none)
             | jnp.where(key + 1 > pos, jnp.uint32(0xFFFF0000), none))
    for x in range(GH):
        msk[pl.ds(M_OLD + n * x, n), :] = jnp.where(band < x, full, jnp.where(band == x, newer, none))
        msk[pl.ds(M_NEW + n * x, n), :] = jnp.where(band > x, full, jnp.where(band == x, ~newer, none))

    def project(w_ref, w0, rows, x, slot, pause=False):
        wrows = pl.ds(w0, rows // 2)
        tail[slot, 0:rows, :] = _mm(_bf16(w_ref[wrows, DM:D]),
                                    jnp.concatenate([x(DM, D - DM, t) for t in range(NT)], axis=1))
        if pause:
            yield None
        for t in range(NT):
            yield _mm(_bf16(w_ref[wrows, 0:DM]), x(0, DM, t)) + tail[slot, 0:rows, t * 128:(t + 1) * 128]

    def key_table(slot):
        for x in range(2):
            k = kf[pl.ds(SLOT_KEY[slot] + x, 8, stride=2), :]
            for d in range(DH):
                kd = jnp.broadcast_to(k[:, d:d + 1], (8, 128))
                for t in range(DUP):
                    ktab[t, slot, _tslot(x, d)] = kd

    for cp in (wq_copy, wk_copy, wv_copy):
        cp.wait()
    x_copy(1).start()
    x_copy(2).start()
    wat[24:, :] = pltpu.bitcast(wsq[0].T, U32)
    pad = jnp.zeros((24 - DH, D), F32)
    wat[0:24, :] = _pack(jnp.concatenate([wk[...].astype(F32), pad, wv[...].astype(F32), pad], axis=0))

    for c in range(NB):
        if c == 0:
            x_copy(0).wait()
            x_copy(3).start()
            wqkv_copy.start()
        if c == 1:
            x_copy(1).wait()
            x_copy(2).wait()
            xb_copy.start()
        if c == 3:
            x_copy(3).wait()
            wqkv_copy.wait()
            wbt[...] = pltpu.bitcast(wqkv[...].T, U32)
        for slot, k0 in enumerate(SLOT_KEY):
            if k0 // QB == c - 1:
                key_table(slot)
        tiles = project(wat, 0, D + 48, lambda k0, k, t: xa[k0:k0 + k, pl.ds(c * QB + t * 128, 128)], 0)
        for t, r in enumerate(tiles):
            c0 = c * QB + t * 128
            kt = r[0:24]
            vt = r[24:48].astype(BF16).astype(F32)
            row = _iota((24, 128), 0)
            for u in range(GH):
                ku = kt if u == 0 else pltpu.roll(kt, 2 * u, 0)
                ku = jnp.concatenate([ku, jnp.zeros((8, 128), F32)], axis=0).T
                if u == 0:
                    kf[pl.ds(c0, 128), 0:32] = ku
                ka[u, pl.ds(c0 // 2, 64), :] = _pack(ku)
                vu = vt if u == 0 else pltpu.roll(vt, 2 * u, 0)
                va[u, :, pl.ds(c0, 128)] = jnp.where((row >= 2 * u) & (row < 2 * u + DH), vu, 1.0)
            for g in range(NG):
                qa[(c * NG + g) * NT + t] = r[48 + g * GR:48 + (g + 1) * GR] * QSCALE

    for slot, k0 in enumerate(SLOT_KEY):
        if k0 // QB == NB - 1:
            key_table(slot)

    def b_project(p, c):
        zero = jnp.zeros((GP - GR, 128), F32)
        for part in (1, 0, 2):
            tiles = project(wbt, pl.multiple_of(part * (D // 2) + p * GR, 8), 2 * GR,
                            lambda k0, k, t: xb[k0:k0 + k, _tile(c * NT + t)], part, pause=True)
            yield next(tiles)
            for t, r in enumerate(tiles):
                i = c * NT + t
                if part == 2:
                    v, row = r.astype(BF16).astype(F32), _iota((8, 128), 0)
                    for y in range(2 * GH):
                        h, r0 = y % GH, (y // GH) * GR + 16 * (y % GH)
                        if h == 0:
                            win = [v[r0:r0 + 16], jnp.where(row >= 2, 1.0, v[r0 + 16:r0 + 24])]
                        else:
                            win = [jnp.where(row >= 2 * h, v[r0:r0 + 8], 1.0), v[r0 + 8:r0 + 24]]
                        vb[y, :, _tile(i)] = jnp.concatenate(win, axis=0)
                else:
                    for y in range(2):
                        rg = jnp.concatenate([r[y * GR:(y + 1) * GR], zero], axis=0)
                        if part == 0:
                            qb[y, :, _tile(i)] = _pack(rg * QSCALE)
                        else:
                            kb[y, pl.ds(pl.multiple_of(i * 64, 64), 64), :] = pltpu.bitcast(rg.astype(BF16).T, U32)
                yield

    def b_scores(y, i, after):
        q = qb[y, :, _tile(i)]
        q = jnp.concatenate([after(q[8 * r:8 * r + 8]) for r in range(GP // 16)], axis=0)
        e0 = (i % 2) * (BR // 2)
        first = max(0, 8 - 4 * i)
        keys = lambda r, m: kb[y, pl.ds(64 * (i - 2) + r, m), :]
        mid = max(first, GH - 1)
        for t in range(GH):
            band = after(msk[pl.ds(M_KEY + 8 * t, 8), :].astype(jnp.int32))[:, 0:GP]
            ks = [keys(9 * n + 8 * x, 8) if first else
                  jnp.where(band > x // 2, keys(9 * n + 8 * x, 8), keys(8 * x, 8)) for x in range(2 * (GH - 1))]
            ks.append(keys(mid * n, (9 - mid) * n))
            s = _mm(_bf16(jnp.concatenate(ks, axis=0)),
                    _bf16(q & msk[pl.ds(M_QUERY + t * (GP // 2), GP // 2), :]))
            if first:
                eb[e0:e0 + 3 * n, _tile(t)] = _pack(jnp.exp2(s[0:3 * BAND]))
                eb[e0 + mid * n:e0 + 9 * n, _tile(t)] = _pack(jnp.exp2(s[3 * BAND:]))
            else:
                eb[e0:e0 + 9 * n, _tile(t)] = _pack(jnp.exp2(s))
        return s

    def b_unskew(i, x, after):
        e0 = (i % 2) * (BR // 2)
        band = after(_iota((8, 128), 1) >> 5)
        band = jnp.concatenate([band, band], axis=0)
        odd_band, high_band = (band & 1) == 1, band >= 2
        out = [[] for _ in range(GH)]
        for blk in range(4 * x, 4 * x + 4):
            src = [eb[pl.ds(e0 + (blk % 9) * n, n), _tile(t)] for t in range(GH)]
            if blk == 0:
                res = src
            elif blk == 11:
                res = [src[(h - 3) % GH] for h in range(GH)]
            else:
                res = [jnp.where(odd_band, src[(h - 1) % GH], src[h]) for h in range(GH)]
                if blk == 10:
                    res = [res[(h - 2) % GH] for h in range(GH)]
                elif blk > 1:
                    res = [jnp.where(high_band, res[(h - 2) % GH], res[h]) for h in range(GH)]
            if x != 1:
                mask = msk[pl.ds(M_OLD + n * blk if x == 0 else M_NEW + n * (blk - 8), n), :]
                res = [r & mask for r in res]
            for h in range(GH):
                out[h].append(res[h])
        return [_bf16(jnp.concatenate(o, axis=0)) for o in out]

    def b_store(p, y, i, outs):
        ob[pl.ds(pl.multiple_of((2 * p + y) * GR, 8), GR), _tile(i)] = _stitch(outs)

    def b_output(p, y, i, z, pause=lambda: None, after=lambda x: lambda v: v):
        outs = [None] * GH
        for x in range(3):
            if i + x >= 2:
                for h, e in enumerate(b_unskew(i, x, after(x))):
                    a = _mm(vb[y * GH + h, :, _tile(i + x - 2)], e)
                    outs[h] = a if outs[h] is None else outs[h] + a
            pause()
        for h in range(GH):
            outs[h], z = _normalise(outs[h], h, z)
        b_store(p, y, i, outs)
        return z

    def b_step(p, z):
        @pl.when(p == 1)
        def _():
            woa_copy.wait()
            wob_copy.wait()

        w = jnp.minimum(p, 2)
        wot[pl.ds(pl.multiple_of(w * (D // 2), 8), D // 2), :] = pltpu.bitcast(wsq[w].T, U32)
        always = _always(p)

        def after(dep, row):
            if dep is None:
                return lambda v: v
            row = min(row, dep.shape[0] - 8)
            return lambda v: jnp.where(always, v, pltpu.bitcast(dep[row:row + 8], v.dtype))

        proj, s, prev = b_project(p, 0), None, None
        z = b_output(jnp.maximum(p - 1, 0), 1, NB * NT - 1, z, lambda: next(proj))
        for c in range(NB):
            for _ in proj:
                pass
            proj = b_project(p, c + 1) if c + 1 < NB else iter(())
            rows = (0, 160, 280, 280) if c + 1 < NB else (0, 40, 80, 160)
            for y in range(2):
                for i in range(c * NT, (c + 1) * NT):
                    s = b_scores(y, i, after(s, rows[3]))
                    pauses = iter([True, True, False])
                    pause = lambda: next(pauses) and next(proj, None)
                    if prev:
                        z = b_output(p, *prev, z, pause, lambda x: after(s, rows[x]))
                    else:
                        pause()
                    prev = (y, i)
        return z

    xb_copy.wait()
    woa_copy.start()
    wob_copy.start()
    z = jnp.zeros((8, 128), F32)
    z = lax.fori_loop(0, NG // 2, b_step, z)
    z = b_output(NG // 2 - 1, 1, NB * NT - 1, z)

    def a_stage(j, u):
        for t in range(NT):
            qs[u, t, 0:24, :] = qa[j * NT + t, 16 * u:16 * u + 24, :]

    def a_query(u):
        q = jnp.concatenate([qs[u, t, 0:24, :] for t in range(NT)], axis=1)
        return jnp.concatenate([q, jnp.zeros((8, QB), F32)], axis=0).astype(BF16)

    def a_store(j, u, acc):
        oa[(j % NG) * GH + u, :, pl.ds(pl.multiple_of((j // NG) * QB, QB), QB)] = acc

    def a_output(j, u):
        acc = None
        for c in range(NC):
            p = pa[pl.ds(((u % 2) * S + c * KC) // 2, KC // 2), :]
            a = _mm(va[u, :, _tile(c)], _bf16(p))
            acc = a if acc is None else acc + a
            if c == NC - 1:
                a_store(j, u, acc)
            yield

    def a_step(jj, _):
        vpu = _VpuScores(jj)
        for y in range(AU):
            j = jj * AU + y
            for u in range(GH):
                pv = a_output(jnp.maximum(j - 1, 0), GH - 1) if u == 0 else a_output(j, u - 1)
                p0, q, slot = (u % 2) * (S // 2), a_query(u), 0
                for c in range(NC):
                    next(pv)
                    m = (KC - 16 * SLOTS[c]) // 2
                    s = _mm(_bf16(ka[u, pl.ds(c * (KC // 2), m), :]), q)
                    pa[pl.ds(p0 + c * (KC // 2), m), :] = _pack(jnp.exp2(s))
                    while slot < NS and slot * NC < (c + 1) * NS:
                        for t in range(NT):
                            pa[pl.ds(p0 + SLOT_KEY[slot] // 2, 8), _tile(t)] = vpu(
                                lambda x, d: ktab[t % DUP, slot, _tslot(x, d)],
                                lambda d: qs[u, t, pl.ds(2 * u + d, 8, stride=0), :])
                        slot += 1
                a_stage(jnp.minimum(j + 1, NB * NG - 1), u)
        return 0

    for u in range(GH):
        a_stage(0, u)
    lax.fori_loop(0, NB * NG // AU, a_step, 0)
    for _ in a_output(NB * NG - 1, GH - 1):
        pass

    def out_copy(i):
        return pltpu.make_async_copy(obuf.at[_tile(i), :], out_hbm.at[_tile(i), :], out_sem.at[i])

    def proj_o(c, z):
        late = jnp.maximum(c * NT - 1, 0)
        obuf[_tile(late), :] = _bf16(ybuf[...]).T
        xs = []
        for t in range(NT):
            groups = []
            for g in range(NG):
                outs = []
                for u in range(GH):
                    o, z = _normalise(oa[g * GH + u, :, _tile(c * NT + t)], u, z)
                    outs.append(o)
                groups.append(_stitch(outs))
            xs.append(jnp.concatenate(groups, axis=0))
        yb = project(wot, D, D, lambda k0, k, t: ob[k0:k0 + k, _tile(c * NT + t)].astype(BF16), 1)
        ya = project(wot, D // 2, D, lambda k0, k, t: xs[t][k0:k0 + k].astype(BF16), 0)
        for t, (b, a) in enumerate(zip(yb, ya)):
            y = jnp.concatenate([a, b], axis=0)
            if t < NT - 1:
                obuf[_tile(c * NT + t), :] = y.astype(BF16).T
                out_copy(c * NT + t).start()
            else:
                ybuf[...] = _pack(y)

        @pl.when(c > 0)
        def _():
            out_copy(late).start()
        return z

    def finish(z):
        z = lax.fori_loop(0, NB, proj_o, z)
        obuf[_tile(NB * NT - 1), :] = _bf16(ybuf[...]).T
        out_copy(NB * NT - 1).start()
        for i in range(NB * NT):
            out_copy(i).wait()
        return z

    z = finish(z)

    unsafe = jnp.max(jnp.where(z < 2.0 ** 120, 0, 1))

    @pl.when(unsafe > 0)
    def _():
        def a_exact(j, _):
            for u in range(GH):
                a_stage(j, u)
                q = a_query(u)

                def scores(c):
                    return _mm(_bf16(ka[u, pl.ds(pl.multiple_of(c * (KC // 2), KC // 2), KC // 2), :]), q)

                m = lax.fori_loop(
                    0, NC, lambda c, m: jnp.maximum(m, jnp.max(scores(c), axis=0, keepdims=True)),
                    jnp.full((1, QB), -jnp.inf, F32))
                acc = lax.fori_loop(
                    0, NC, lambda c, acc: acc + _mm(va[u, :, _tile(c)], jnp.exp2(scores(c) - m).astype(BF16)),
                    jnp.zeros((24, QB), F32))
                a_store(j, u, acc)
            return 0

        def b_exact(p, _):
            def project_block(c, _):
                for _ in b_project(p, c):
                    pass
                return 0

            def attend(step, _):
                y, i = step // (NB * NT), step % (NB * NT)
                k0 = jnp.maximum(i - 2, 0)
                q = qb[y, :, _tile(i)]
                k = _bf16(kb[y, pl.ds(pl.multiple_of(k0 * 64, 64), 192), :])
                dist = _iota((384, 128), 1) - _iota((384, 128), 0) + (i - k0) * 128
                keep = (dist >= 0) & (dist < W)
                row = _iota(q.shape, 0)
                qh = [jnp.where((row >= h * (DH // 2)) & (row < (h + 1) * (DH // 2)), q, none) for h in range(GH)]
                s4 = _mm(k, _bf16(jnp.concatenate(qh, axis=1)))
                outs = []
                for h in range(GH):
                    s = jnp.where(keep, s4[:, h * 128:(h + 1) * 128], NEG)
                    e = jnp.exp2(s - jnp.max(s, axis=0, keepdims=True)).astype(BF16)
                    v = vb[y * GH + h, :, pl.ds(pl.multiple_of(k0 * 128, 128), 384)]
                    outs.append(_normalise(_mm(v, e), h, z)[0])
                b_store(p, y, i, outs)
                return 0

            lax.fori_loop(0, NB, project_block, 0)
            lax.fori_loop(0, 2 * NB * NT, attend, 0)
            return 0

        lax.fori_loop(0, NB * NG, a_exact, 0)
        lax.fori_loop(0, NG // 2, b_exact, 0)
        finish(z)


@jax.jit
def pallas_concat_heads__grouped_kv_mqa__sliding_block__prompt_kernel(
    A_x: jax.Array,
    A_wq: jax.Array,
    A_wk: jax.Array,
    A_wv: jax.Array,
    A_wo: jax.Array,
    B_x: jax.Array,
    B_wqkv: jax.Array,
    B_wo: jax.Array,
):
    hbm = pl.BlockSpec(memory_space=pltpu.HBM)
    vmem = pltpu.VMEM
    out = pl.pallas_call(
        _kernel,
        in_specs=[hbm] * 8,
        out_specs=hbm,
        out_shape=jax.ShapeDtypeStruct((S, 2 * D), BF16),
        scratch_shapes=[
            vmem((D, S), BF16), vmem((3, D, D), BF16), vmem((DH, D), BF16), vmem((DH, D), BF16),
            vmem((D, S), BF16), vmem((D, 3 * D), BF16),
            vmem((D // 2 + 24, D), U32), vmem((3 * D // 2, D), U32), vmem((3 * D // 2, D), U32),
            vmem((3, D + 48, QB), F32),
            vmem((NB * NG * NT, GR, 128), F32), vmem((GH, NT, 32, 128), F32), vmem((GH, S // 2, 32), U32),
            vmem((S, 128), F32), vmem((GH, 24, S), F32), vmem((DUP, NS, TROWS, 8, 128), F32),
            vmem((S, QB), U32), vmem((H, 24, S), F32),
            vmem((2, GP // 2, S), U32), vmem((2, S // 2, GP), U32), vmem((2 * GH, 24, S), F32),
            vmem((BR, QB), U32), vmem((D, S), F32), vmem((M_ROWS, 128), U32),
            vmem((D, 128), U32), vmem((S, 2 * D), BF16),
            pltpu.SemaphoreType.DMA((7,)), pltpu.SemaphoreType.DMA((NB,)),
            pltpu.SemaphoreType.DMA((NB * NT,)),
        ],
        compiler_params=pltpu.CompilerParams(vmem_limit_bytes=100 * 1024 * 1024),
        name="mqa_swa_fused",
    )(A_x[0].T, A_wq, A_wk.T, A_wv.T, A_wo, B_x[0].T, B_wqkv, B_wo)
    return out[None]
```

```python
import math

import jax
import jax.numpy as jnp
from jax import lax
import jax.experimental.pallas as pl
import jax.experimental.pallas.tpu as pltpu

S = 2048
D = 576
H = 32
DH = D // H
W = 256
F32 = jnp.float32
BF16 = jnp.bfloat16
U32 = jnp.uint32
LOG2E = math.log2(math.e)
QSCALE = (DH ** -0.5) * LOG2E
NEG = -1e9 * LOG2E

QB = 512
NB = S // QB
NT = QB // 128
KC = 128
NC = S // KC
GH = 4
NG = H // GH
GR = GH * DH
GP = 80
BAND = 32
BR = W + BAND
DM = D // 128 * 128
LATE = DM + 128

NS = 19
SLOTS = [(NS * (c + 1)) // 12 - (NS * c) // 12 if c < 12 else 0 for c in range(NC)]
SLOT_KEY = [(c + 1) * KC - 16 * (SLOTS[c] - x) for c in range(NC) for x in range(SLOTS[c])]
A_UNROLL = 2

M_QUERY, M_OLD, M_NEW, M_KEY, M_ROWS = 0, 160, 224, 288, 320


def _mm(a, b):
    return lax.dot_general(a, b, (((1,), (0,)), ((), ())), preferred_element_type=F32)


def _pack(x):
    return pltpu.bitcast(x.astype(BF16), U32)


def _bf16(x):
    return pltpu.bitcast(x, BF16)


def _iota(shape, dim):
    return lax.broadcasted_iota(jnp.int32, shape, dim)


def _tile(i):
    return pl.ds(pl.multiple_of(i * 128, 128), 128)


def _always(step):
    return _iota((8, 128), 0) <= step + 8


class _VpuScores:
    def __init__(self, step):
        self.always, self.count, self.release, self.stored = _always(step), 0, None, None
        self.always2 = jnp.concatenate([self.always] * 2, axis=0)

    def __call__(self, keys, query, out_ref):
        n, wait = self.count, self.release
        for d in range(DH):
            term = keys(d) * query(d)
            if d == 0 and n:
                term = jnp.where(self.always2, term, wait)
            if d == 10 and n:
                term = jnp.concatenate([jnp.where(self.always, term[0:8], self.stored), term[8:16]], axis=0)
            acc = term if d == 0 else acc + term
            if d == 13 + n % 2:
                self.release = acc
        out_ref[...] = _pack(jnp.exp2(acc))
        self.count, self.stored = n + 1, pltpu.bitcast(out_ref[...], F32)


def _normalise(acc, u, z):
    den = acc[23:24] if u == 0 else acc[0:1]
    r = pltpu.reciprocal(den, approx=True)
    r = r * (2.0 - den * r)
    big = r * (2.0 ** 20)
    sq = acc * acc
    return acc * r, z + (sq[0:8] + sq[8:16] + sq[16:24] + big * big)


def _stitch(outs):
    row = _iota((8, 128), 0)
    rows = [outs[0][0:16]]
    for h in range(1, GH):
        rows.append(jnp.where(row >= 2 * h, outs[h][0:8], outs[h - 1][16:24]))
        rows.append(outs[h][8:16])
    rows.append(outs[GH - 1][16:24])
    return jnp.concatenate(rows, axis=0)


def _kernel(xa_hbm, wq_hbm, wk_hbm, wv_hbm, woa_hbm, xb_hbm, wqkv_hbm, wob_hbm,
            out_hbm,
            xa, wq, wk, wv, xb, wqkv, wo,
            wat, wbt, wot, atail, tail,
            qa, qs, ka, kf, va, ktab, pa, oa,
            qb, kb, vb, eb, ob, msk,
            ybuf, obuf, in_sem, out_sem):

    head, rest = pl.ds(0, DM), pl.ds(DM, D - DM)
    pairs = [(wq_hbm.at[rest], wq.at[rest]), (xa_hbm.at[rest], xa.at[rest]), (wk_hbm, wk), (wv_hbm, wv),
             (wq_hbm.at[head], wq.at[head]), (wqkv_hbm, wqkv),
             (xb_hbm, xb), (woa_hbm, wo.at[0]), (wob_hbm, wo.at[1])]
    pairs += [(xa_hbm.at[head, pl.ds(c * QB, QB)], xa.at[head, pl.ds(c * QB, QB)]) for c in range(NB)]
    copies = [pltpu.make_async_copy(src, dst, in_sem.at[i]) for i, (src, dst) in enumerate(pairs)]
    first_copies, (wq_copy, wqkv_copy), late_copies, x_copies = copies[:4], copies[4:6], copies[6:9], copies[9:]

    for cp in first_copies + [wq_copy]:
        cp.start()

    ones = jnp.uint32(0x3F803F80)
    pa[S // 2:, :] = jnp.full((S // 2, QB), ones, U32)
    eb[BR // 2:, :] = jnp.full((BR // 2, QB), ones, U32)
    vb[GH:, :, S - 384:] = jnp.ones((GH, 24, 384), F32)
    ybuf[...] = jnp.full(ybuf.shape, ones, U32)
    obuf[S:, 0:128] = jnp.zeros((32, 128), BF16)

    n, full, none = BAND // 2, jnp.uint32(0xFFFFFFFF), jnp.uint32(0)
    for t in range(GH):
        owner = ((_iota((GP // 2, 128), 1) >> 5) + t) & (GH - 1)
        row = _iota((GP // 2, 128), 0)
        msk[pl.ds(M_QUERY + t * (GP // 2), GP // 2), :] = jnp.where(
            (row >= owner * (DH // 2)) & (row < (owner + 1) * (DH // 2)), full, none)
        lane_head = sum(jnp.where(_iota((8, 128), 1) >= x * DH, 1, 0) for x in range(1, GH))
        msk[pl.ds(M_KEY + 8 * t, 8), :] = ((lane_head + (GH - t)) & (GH - 1)).astype(U32)
    lane = _iota((n, 128), 1)
    band, pos, key = lane >> 5, lane & (BAND - 1), 2 * _iota((n, 128), 0)
    newer = (jnp.where(key > pos, jnp.uint32(0xFFFF), none)
             | jnp.where(key + 1 > pos, jnp.uint32(0xFFFF0000), none))
    for x in range(GH):
        msk[pl.ds(M_OLD + n * x, n), :] = jnp.where(band < x, full, jnp.where(band == x, newer, none))
        msk[pl.ds(M_NEW + n * x, n), :] = jnp.where(band > x, full, jnp.where(band == x, ~newer, none))

    def project(w_ref, w0, rows, x, slot, pause=False):
        wrows = pl.ds(w0, rows // 2)
        tail[slot, 0:rows, :] = _mm(_bf16(w_ref[wrows, DM:D]),
                                    jnp.concatenate([x(DM, D - DM, t) for t in range(NT)], axis=1))
        if pause:
            yield None
        for t in range(NT):
            yield _mm(_bf16(w_ref[wrows, 0:DM]), x(0, DM, t)) + tail[slot, 0:rows, t * 128:(t + 1) * 128]

    def key_table(slot):
        k = kf[pl.ds(SLOT_KEY[slot], 16), :]
        for d in range(DH):
            ktab[0, slot, pl.ds(16 * d, 16), :] = jnp.broadcast_to(k[:, d:d + 1], (16, 128))

    for cp in first_copies:
        cp.wait()
    x_copies[0].start()
    pad = jnp.zeros((24 - DH, D), F32)
    wat[0:24, :] = _pack(jnp.concatenate([wk[...].astype(F32), pad, wv[...].astype(F32), pad], axis=0))
    wat[24:, rest] = pltpu.bitcast(wq[rest, :].T, U32)
    for c in range(NB):
        if c == NB // 2:
            wq_copy.wait()
            x_copies[1].start()
            wat[24:, head] = pltpu.bitcast(wq[head, :].T, U32)
        atail[:, pl.ds(c * QB, QB)] = _mm(_bf16(wat[:, rest]), xa[rest, pl.ds(c * QB, QB)])

    for c in range(NB):
        if c == 0:
            x_copies[0].wait()
            for cp in x_copies[2:] + [wqkv_copy]:
                cp.start()
        if c == 1:
            x_copies[1].wait()
            x_copies[2].wait()
        if c == 3:
            x_copies[3].wait()
            wqkv_copy.wait()
            for cp in late_copies:
                cp.start()
            wbt[...] = pltpu.bitcast(wqkv[...].T, U32)
        for slot, k0 in enumerate(SLOT_KEY):
            if k0 // QB == c - 1:
                key_table(slot)
        for t in range(NT):
            c0 = c * QB + t * 128
            r = _mm(_bf16(wat[:, head]), xa[head, pl.ds(c0, 128)]) + atail[:, pl.ds(c0, 128)]
            kt = r[0:24]
            vt = r[24:48].astype(BF16).astype(F32)
            row = _iota((24, 128), 0)
            for u in range(GH):
                ku = kt if u == 0 else pltpu.roll(kt, 2 * u, 0)
                ku = jnp.concatenate([ku, jnp.zeros((8, 128), F32)], axis=0).T
                if u == 0:
                    kf[pl.ds(c0, 128), :] = ku
                ka[u, pl.ds(c0 // 2, 64), :] = _pack(ku)
                vu = vt if u == 0 else pltpu.roll(vt, 2 * u, 0)
                va[u, :, pl.ds(c0, 128)] = jnp.where((row >= 2 * u) & (row < 2 * u + DH), vu, 1.0)
            qa[:, pl.ds(c0, 128)] = r[48:] * QSCALE

    def b_project(p, c):
        zero = jnp.zeros((GP - GR, 128), F32)
        for part in (1, 0, 2):
            tiles = project(wbt, pl.multiple_of(part * (D // 2) + p * GR, 8), 2 * GR,
                            lambda k0, k, t: xb[k0:k0 + k, _tile(c * NT + t)], part, pause=True)
            yield next(tiles)
            for t, r in enumerate(tiles):
                i = c * NT + t
                if part == 2:
                    v, row = r.astype(BF16).astype(F32), _iota((8, 128), 0)
                    for y in range(2 * GH):
                        h, r0 = y % GH, (y // GH) * GR + 16 * (y % GH)
                        if h == 0:
                            win = [v[r0:r0 + 16], jnp.where(row >= 2, 1.0, v[r0 + 16:r0 + 24])]
                        else:
                            win = [jnp.where(row >= 2 * h, v[r0:r0 + 8], 1.0), v[r0 + 8:r0 + 24]]
                        vb[y, :, _tile(i)] = jnp.concatenate(win, axis=0)
                else:
                    for y in range(2):
                        rg = jnp.concatenate([r[y * GR:(y + 1) * GR], zero], axis=0)
                        if part == 0:
                            qb[y, :, _tile(i)] = _pack(rg * QSCALE)
                        else:
                            kb[y, pl.ds(pl.multiple_of(i * 64, 64), 64), :] = pltpu.bitcast(rg.astype(BF16).T, U32)
                yield

    def b_scores(y, i, after):
        q = qb[y, :, _tile(i)]
        q = jnp.concatenate([after(q[8 * r:8 * r + 8]) for r in range(GP // 16)], axis=0)
        e0 = (i % 2) * (BR // 2)
        first = max(0, 8 - 4 * i)
        keys = lambda r, m: kb[y, pl.ds(64 * (i - 2) + r, m), :]
        mid = max(first, GH - 1)
        for t in range(GH):
            band = after(msk[pl.ds(M_KEY + 8 * t, 8), :].astype(jnp.int32))[:, 0:GP]
            ks = [keys(9 * n + 8 * x, 8) if first else
                  jnp.where(band > x // 2, keys(9 * n + 8 * x, 8), keys(8 * x, 8)) for x in range(2 * (GH - 1))]
            ks.append(keys(mid * n, (9 - mid) * n))
            s = _mm(_bf16(jnp.concatenate(ks, axis=0)),
                    _bf16(q & msk[pl.ds(M_QUERY + t * (GP // 2), GP // 2), :]))
            if first:
                eb[e0:e0 + 3 * n, _tile(t)] = _pack(jnp.exp2(s[0:3 * BAND]))
                eb[e0 + mid * n:e0 + 9 * n, _tile(t)] = _pack(jnp.exp2(s[3 * BAND:]))
            else:
                eb[e0:e0 + 9 * n, _tile(t)] = _pack(jnp.exp2(s))
        return s

    def b_unskew(i, x, after):
        e0 = (i % 2) * (BR // 2)
        band = after(_iota((8, 128), 1) >> 5)
        band = jnp.concatenate([band, band], axis=0)
        odd_band, high_band = (band & 1) == 1, band >= 2
        out = [[] for _ in range(GH)]
        for blk in range(4 * x, 4 * x + 4):
            src = [eb[pl.ds(e0 + (blk % 9) * n, n), _tile(t)] for t in range(GH)]
            if blk == 0:
                res = src
            elif blk == 11:
                res = [src[(h - 3) % GH] for h in range(GH)]
            else:
                res = [jnp.where(odd_band, src[(h - 1) % GH], src[h]) for h in range(GH)]
                if blk == 10:
                    res = [res[(h - 2) % GH] for h in range(GH)]
                elif blk > 1:
                    res = [jnp.where(high_band, res[(h - 2) % GH], res[h]) for h in range(GH)]
            if x != 1:
                mask = msk[pl.ds(M_OLD + n * blk if x == 0 else M_NEW + n * (blk - 8), n), :]
                res = [r & mask for r in res]
            for h in range(GH):
                out[h].append(res[h])
        return [_bf16(jnp.concatenate(o, axis=0)) for o in out]

    def b_store(p, y, i, outs):
        ob[pl.ds(pl.multiple_of((2 * p + y) * GR, 8), GR), _tile(i)] = _stitch(outs)

    def b_output(p, y, i, z, pause=lambda: None, after=lambda x: lambda v: v):
        outs = [None] * GH
        for x in range(3):
            if i + x >= 2:
                for h, e in enumerate(b_unskew(i, x, after(x))):
                    a = _mm(vb[y * GH + h, :, _tile(i + x - 2)], e)
                    outs[h] = a if outs[h] is None else outs[h] + a
            pause()
        for h in range(GH):
            outs[h], z = _normalise(outs[h], h, z)
        b_store(p, y, i, outs)
        return z

    def b_step(p, z):
        w = p % 2
        wot[pl.ds(pl.multiple_of(w * (D // 2), 8), D // 2), :] = pltpu.bitcast(wo[w].T, U32)
        always = _always(p)

        def after(dep, row):
            if dep is None:
                return lambda v: v
            row = min(row, dep.shape[0] - 8)
            return lambda v: jnp.where(always, v, pltpu.bitcast(dep[row:row + 8], v.dtype))

        proj, s, prev = b_project(p, 0), None, None
        z = b_output(jnp.maximum(p - 1, 0), 1, NB * NT - 1, z, lambda: next(proj))
        for c in range(NB):
            for _ in proj:
                pass
            proj = b_project(p, c + 1) if c + 1 < NB else iter(())
            rows = (0, 160, 280, 280) if c + 1 < NB else (0, 40, 80, 160)
            for y in range(2):
                for i in range(c * NT, (c + 1) * NT):
                    s = b_scores(y, i, after(s, rows[3]))
                    pauses = iter([True, True, False])
                    pause = lambda: next(pauses) and next(proj, None)
                    if prev:
                        z = b_output(p, *prev, z, pause, lambda x: after(s, rows[x]))
                    else:
                        pause()
                    prev = (y, i)
        return z

    def a_stage(j, u):
        qs[u] = qa[pl.ds(pl.multiple_of((j % NG) * GR + 16 * u, 8), 24),
                   pl.ds(pl.multiple_of((j // NG) * QB, QB), QB)]

    def a_query(u):
        return jnp.concatenate([qs[u], jnp.zeros((8, QB), F32)], axis=0).astype(BF16)

    def a_store(j, u, acc):
        oa[(j % NG) * GH + u, :, pl.ds(pl.multiple_of((j // NG) * QB, QB), QB)] = acc

    def a_output(j, u):
        acc = None
        for c in range(NC):
            p = pa[pl.ds(((u % 2) * S + c * KC) // 2, KC // 2), :]
            a = _mm(va[u, :, _tile(c)], _bf16(p))
            acc = a if acc is None else acc + a
            if c == NC - 1:
                a_store(j, u, acc)
            yield

    def a_step(step, _):
        vpu = _VpuScores(step)
        for j, u in [(step * A_UNROLL + y, u) for y in range(A_UNROLL) for u in range(GH)]:
            pv = a_output(jnp.maximum(j - 1, 0), GH - 1) if u == 0 else a_output(j, u - 1)
            p0, q, slot = (u % 2) * (S // 2), a_query(u), 0
            for c in range(NC):
                next(pv)
                m = (KC - 16 * SLOTS[c]) // 2
                s = _mm(_bf16(ka[u, pl.ds(c * (KC // 2), m), :]), q)
                pa[pl.ds(p0 + c * (KC // 2), m), :] = _pack(jnp.exp2(s))
                while slot < NS and slot * NC < (c + 1) * NS:
                    for t in range(NT):
                        vpu(lambda d: ktab[0, slot, pl.ds(16 * d, 16), :],
                            lambda d: qs[u, pl.ds(2 * u + d, 1), t * 128:(t + 1) * 128],
                            pa.at[pl.ds(p0 + SLOT_KEY[slot] // 2, 8), t * 128:(t + 1) * 128])
                    slot += 1
            a_stage(jnp.minimum(j + 1, NB * NG - 1), u)
        return 0

    for u in range(GH):
        a_stage(0, u)
    lax.fori_loop(0, NB * NG // A_UNROLL, a_step, 0)
    for cp in late_copies:
        cp.wait()
    z = lax.fori_loop(0, NG // 2, b_step, jnp.zeros((8, 128), F32))
    z = b_output(NG // 2 - 1, 1, NB * NT - 1, z)
    for _ in a_output(NB * NG - 1, GH - 1):
        pass

    def attend_exact():
        def a_exact(j, _):
            for u in range(GH):
                a_stage(j, u)
                q = a_query(u)

                def scores(c):
                    return _mm(_bf16(ka[u, pl.ds(pl.multiple_of(c * (KC // 2), KC // 2), KC // 2), :]), q)

                m = lax.fori_loop(
                    0, NC, lambda c, m: jnp.maximum(m, jnp.max(scores(c), axis=0, keepdims=True)),
                    jnp.full((1, QB), -jnp.inf, F32))
                acc = lax.fori_loop(
                    0, NC, lambda c, acc: acc + _mm(va[u, :, _tile(c)], jnp.exp2(scores(c) - m).astype(BF16)),
                    jnp.zeros((24, QB), F32))
                a_store(j, u, acc)
            return 0

        def b_exact(p, _):
            def project_block(c, _):
                for _ in b_project(p, c):
                    pass
                return 0

            def attend(step, _):
                y, i = step // (NB * NT), step % (NB * NT)
                k0 = jnp.maximum(i - 2, 0)
                q = qb[y, :, _tile(i)]
                k = _bf16(kb[y, pl.ds(pl.multiple_of(k0 * 64, 64), 192), :])
                dist = _iota((384, 128), 1) - _iota((384, 128), 0) + (i - k0) * 128
                keep = (dist >= 0) & (dist < W)
                row = _iota(q.shape, 0)
                qh = [jnp.where((row >= h * (DH // 2)) & (row < (h + 1) * (DH // 2)), q, none) for h in range(GH)]
                s4 = _mm(k, _bf16(jnp.concatenate(qh, axis=1)))
                outs = []
                for h in range(GH):
                    s = jnp.where(keep, s4[:, h * 128:(h + 1) * 128], NEG)
                    e = jnp.exp2(s - jnp.max(s, axis=0, keepdims=True)).astype(BF16)
                    v = vb[y * GH + h, :, pl.ds(pl.multiple_of(k0 * 128, 128), 384)]
                    outs.append(_normalise(_mm(v, e), h, z)[0])
                b_store(p, y, i, outs)
                return 0

            lax.fori_loop(0, NB, project_block, 0)
            lax.fori_loop(0, 2 * NB * NT, attend, 0)
            return 0

        lax.fori_loop(0, NB * NG, a_exact, 0)
        lax.fori_loop(0, NG // 2, b_exact, 0)

    def out_copy(i):
        return pltpu.make_async_copy(obuf.at[_tile(i), :], out_hbm.at[_tile(i), :], out_sem.at[i])

    def proj_o(c, z):
        always, spare, started = _always(c), pl.multiple_of(S + 16 * jnp.minimum(c, 0), 16), {}

        def mark(t):
            obuf[pl.ds(spare, 16), 0:128] = jnp.zeros((16, 128), BF16)
            started[t] = pltpu.bitcast(obuf[pl.ds(spare + 16, 16), 0:128], F32)

        def b_tile(k0, k, t):
            x = ob[k0:k0 + k, _tile(c * NT + t)]
            if k0 == 0 and t in started:
                x = jnp.concatenate([jnp.where(always, x[r:r + 8], started[t]) if r % 64 == 0 else x[r:r + 8]
                                     for r in range(0, k, 8)], axis=0)
            return x.astype(BF16)

        late = jnp.maximum(c * NT - 1, 0)
        obuf[_tile(late), 0:LATE] = _bf16(ybuf[...]).T

        @pl.when(c > 0)
        def _():
            out_copy(late).start()

        mark(1)
        xs = []
        for t in range(NT):
            groups = []
            for g in range(NG):
                outs = []
                for u in range(GH):
                    o, z = _normalise(oa[g * GH + u, :, _tile(c * NT + t)], u, z)
                    outs.append(o)
                groups.append(_stitch(outs))
            xs.append(jnp.concatenate(groups, axis=0))
        yb = project(wot, D // 2, D, b_tile, 1)
        ya = project(wot, 0, D, lambda k0, k, t: xs[t][k0:k0 + k].astype(BF16), 0)
        for t, (b, a) in enumerate(zip(yb, ya)):
            y = jnp.concatenate([a, b], axis=0)
            if t < NT - 1:
                obuf[_tile(c * NT + t), :] = y.astype(BF16).T
                out_copy(c * NT + t).start()
                if t + 2 < NT:
                    mark(t + 2)
            else:
                obuf[_tile(c * NT + t), LATE:] = y[LATE:].astype(BF16).T
                ybuf[...] = _pack(y[:LATE])
        return z

    def finish(exact):
        pl.when(exact == 1)(attend_exact)
        check = lax.fori_loop(0, NB, proj_o, z)
        obuf[_tile(NB * NT - 1), 0:LATE] = _bf16(ybuf[...]).T
        out_copy(NB * NT - 1).start()
        unsafe = jnp.max(jnp.where(check < 2.0 ** 120, 0, 1))
        for i in range(NB * NT):
            out_copy(i).wait()
        return jnp.where(unsafe > 0, exact + 1, 2)

    lax.while_loop(lambda exact: exact < 2, finish, jnp.int32(0))


@jax.jit
def pallas_concat_heads__grouped_kv_mqa__sliding_block__prompt_kernel(
    A_x: jax.Array,
    A_wq: jax.Array,
    A_wk: jax.Array,
    A_wv: jax.Array,
    A_wo: jax.Array,
    B_x: jax.Array,
    B_wqkv: jax.Array,
    B_wo: jax.Array,
):
    hbm = pl.BlockSpec(memory_space=pltpu.HBM)
    vmem = pltpu.VMEM
    out = pl.pallas_call(
        _kernel,
        in_specs=[hbm] * 8,
        out_specs=hbm,
        out_shape=jax.ShapeDtypeStruct((S, 2 * D), BF16),
        scratch_shapes=[
            vmem((D, S), BF16), vmem((D, D), BF16), vmem((DH, D), BF16), vmem((DH, D), BF16),
            vmem((D, S), BF16), vmem((D, 3 * D), BF16), vmem((2, D, D), BF16),
            vmem((D // 2 + 24, D), U32), vmem((3 * D // 2, D), U32), vmem((D, D), U32),
            vmem((D + 48, S), F32), vmem((3, D, QB), F32),
            vmem((D, S), F32), vmem((GH, 24, QB), F32), vmem((GH, S // 2, 32), U32),
            vmem((S, 32), F32), vmem((GH, 24, S), F32), vmem((1, NS, 16 * DH + 8, 128), F32),
            vmem((S, QB), U32), vmem((H, 24, S), F32),
            vmem((2, GP // 2, S), U32), vmem((2, S // 2, GP), U32), vmem((2 * GH, 24, S), F32),
            vmem((BR, QB), U32), vmem((D, S), F32), vmem((M_ROWS, 128), U32),
            vmem((LATE // 2, 128), U32), vmem((S + 32, 2 * D), BF16),
            pltpu.SemaphoreType.DMA((9 + NB,)), pltpu.SemaphoreType.DMA((NB * NT,)),
        ],
        compiler_params=pltpu.CompilerParams(vmem_limit_bytes=100 * 1024 * 1024),
        name="mqa_swa_fused",
    )(A_x[0].T, A_wq, A_wk.T, A_wv.T, A_wo, B_x[0].T, B_wqkv, B_wo)
    return out[None]
```

```python
import math

import jax
import jax.numpy as jnp
from jax import lax
import jax.experimental.pallas as pl
import jax.experimental.pallas.tpu as pltpu

S = 2048
D = 576
H = 32
DH = D // H
W = 256
F32 = jnp.float32
BF16 = jnp.bfloat16
U32 = jnp.uint32
LOG2E = math.log2(math.e)
QSCALE = (DH ** -0.5) * LOG2E
NEG = -1e9 * LOG2E

QB = 512
NB = S // QB
NT = QB // 128
KC = 128
NC = S // KC
GH = 4
NG = H // GH
GR = GH * DH
GP = 80
BAND = 32
BR = W + BAND
DM = D // 128 * 128
LATE = DM + 128

NS = 19
SLOTS = [(NS * (c + 1)) // 12 - (NS * c) // 12 if c < 12 else 0 for c in range(NC)]
SLOT_KEY = [(c + 1) * KC - 16 * (SLOTS[c] - x) for c in range(NC) for x in range(SLOTS[c])]
A_UNROLL = 2

M_QUERY, M_OLD, M_NEW, M_KEY, M_ROWS = 0, 160, 224, 288, 320


def _mm(a, b):
    return lax.dot_general(a, b, (((1,), (0,)), ((), ())), preferred_element_type=F32)


def _pack(x):
    return pltpu.bitcast(x.astype(BF16), U32)


def _bf16(x):
    return pltpu.bitcast(x, BF16)


def _iota(shape, dim):
    return lax.broadcasted_iota(jnp.int32, shape, dim)


def _tile(i):
    return pl.ds(pl.multiple_of(i * 128, 128), 128)


def _always(step):
    return _iota((8, 128), 0) <= step + 8


class _VpuScores:
    def __init__(self, step):
        self.always, self.count, self.release, self.stored = _always(step), 0, None, None
        self.always2 = jnp.concatenate([self.always] * 2, axis=0)

    def __call__(self, keys, query, out_ref):
        n, wait = self.count, self.release
        for d in range(DH):
            term = keys(d) * query(d)
            if d == 0 and n:
                term = jnp.where(self.always2, term, wait)
            if d == 10 and n:
                term = jnp.concatenate([jnp.where(self.always, term[0:8], self.stored), term[8:16]], axis=0)
            acc = term if d == 0 else acc + term
            if d == 13 + n % 2:
                self.release = acc
        out_ref[...] = _pack(jnp.exp2(acc))
        self.count, self.stored = n + 1, pltpu.bitcast(out_ref[...], F32)


def _normalise(acc, u, z):
    den = acc[23:24] if u == 0 else acc[0:1]
    r = pltpu.reciprocal(den, approx=True)
    r = r * (2.0 - den * r)
    size = jnp.abs(acc)
    return acc * r, z + (size[0:8] + size[8:16] + size[16:24] + r * (2.0 ** 80))


def _stitch(outs):
    row = _iota((8, 128), 0)
    rows = [outs[0][0:16]]
    for h in range(1, GH):
        rows.append(jnp.where(row >= 2 * h, outs[h][0:8], outs[h - 1][16:24]))
        rows.append(outs[h][8:16])
    rows.append(outs[GH - 1][16:24])
    return jnp.concatenate(rows, axis=0)


def _kernel(xa_hbm, wq_hbm, wk_hbm, wv_hbm, woa_hbm, xb_hbm, wqkv_hbm, wob_hbm,
            out_hbm,
            xa, wq, wk, wv, xb, wqkv, wo,
            wat, wbt, wot, atail, tail,
            qa, qs, ka, kf, va, ktab, pa, oa,
            qb, kb, vb, eb, ob, msk,
            ybuf, obuf, in_sem, out_sem):

    head, rest = pl.ds(0, DM), pl.ds(DM, D - DM)
    pairs = [(wq_hbm.at[rest], wq.at[rest]), (xa_hbm.at[rest], xa.at[rest]), (wk_hbm, wk), (wv_hbm, wv),
             (wq_hbm.at[head], wq.at[head]), (wqkv_hbm, wqkv),
             (xb_hbm, xb), (woa_hbm, wo.at[0]), (wob_hbm, wo.at[1])]
    pairs += [(xa_hbm.at[head, pl.ds(c * QB, QB)], xa.at[head, pl.ds(c * QB, QB)]) for c in range(NB)]
    copies = [pltpu.make_async_copy(src, dst, in_sem.at[i]) for i, (src, dst) in enumerate(pairs)]
    first_copies, (wq_copy, wqkv_copy), late_copies, x_copies = copies[:4], copies[4:6], copies[6:9], copies[9:]

    for cp in first_copies + [wq_copy]:
        cp.start()

    ones = jnp.uint32(0x3F803F80)
    pa[S // 2:, :] = jnp.full((S // 2, QB), ones, U32)
    eb[BR // 2:, :] = jnp.full((BR // 2, QB), ones, U32)
    vb[GH:, :, S - 384:] = jnp.ones((GH, 24, 384), F32)
    ybuf[...] = jnp.full(ybuf.shape, ones, U32)
    obuf[S:, 0:128] = jnp.zeros((32, 128), BF16)

    n, full, none = BAND // 2, jnp.uint32(0xFFFFFFFF), jnp.uint32(0)
    for t in range(GH):
        owner = ((_iota((GP // 2, 128), 1) >> 5) + t) & (GH - 1)
        row = _iota((GP // 2, 128), 0)
        msk[pl.ds(M_QUERY + t * (GP // 2), GP // 2), :] = jnp.where(
            (row >= owner * (DH // 2)) & (row < (owner + 1) * (DH // 2)), full, none)
        lane_head = sum(jnp.where(_iota((8, 128), 1) >= x * DH, 1, 0) for x in range(1, GH))
        msk[pl.ds(M_KEY + 8 * t, 8), :] = ((lane_head + (GH - t)) & (GH - 1)).astype(U32)
    lane = _iota((n, 128), 1)
    band, pos, key = lane >> 5, lane & (BAND - 1), 2 * _iota((n, 128), 0)
    newer = (jnp.where(key > pos, jnp.uint32(0xFFFF), none)
             | jnp.where(key + 1 > pos, jnp.uint32(0xFFFF0000), none))
    for x in range(GH):
        msk[pl.ds(M_OLD + n * x, n), :] = jnp.where(band < x, full, jnp.where(band == x, newer, none))
        msk[pl.ds(M_NEW + n * x, n), :] = jnp.where(band > x, full, jnp.where(band == x, ~newer, none))

    def project(w_ref, w0, rows, x, slot, pause=False):
        wrows = pl.ds(w0, rows // 2)
        tail[slot, 0:rows, :] = _mm(_bf16(w_ref[wrows, DM:D]),
                                    jnp.concatenate([x(DM, D - DM, t) for t in range(NT)], axis=1))
        if pause:
            yield None
        for t in range(NT):
            yield _mm(_bf16(w_ref[wrows, 0:DM]), x(0, DM, t)) + tail[slot, 0:rows, t * 128:(t + 1) * 128]

    def key_table(slot):
        k = kf[pl.ds(SLOT_KEY[slot], 16), :]
        for d in range(DH):
            ktab[slot, pl.ds(16 * d, 16), :] = jnp.broadcast_to(k[:, d:d + 1], (16, 128))

    for cp in first_copies:
        cp.wait()
    x_copies[0].start()
    pad = jnp.zeros((24 - DH, D), F32)
    wat[0:24, :] = _pack(jnp.concatenate([wk[...].astype(F32), pad, wv[...].astype(F32), pad], axis=0))
    wat[24:, rest] = pltpu.bitcast(wq[rest, :].T, U32)
    for c in range(NB):
        if c == NB // 2:
            wq_copy.wait()
            x_copies[1].start()
            wat[24:, head] = pltpu.bitcast(wq[head, :].T, U32)
        atail[:, pl.ds(c * QB, QB)] = _mm(_bf16(wat[:, rest]), xa[rest, pl.ds(c * QB, QB)])

    for c in range(NB):
        if c == 0:
            x_copies[0].wait()
            for cp in x_copies[2:] + [wqkv_copy]:
                cp.start()
        if c == 1:
            x_copies[1].wait()
            x_copies[2].wait()
        if c == 3:
            x_copies[3].wait()
            wqkv_copy.wait()
            for cp in late_copies:
                cp.start()
            wbt[...] = pltpu.bitcast(wqkv[...].T, U32)
        for slot, k0 in enumerate(SLOT_KEY):
            if k0 // QB == c - 1:
                key_table(slot)
        for t in range(NT):
            c0 = c * QB + t * 128
            r = _mm(_bf16(wat[:, head]), xa[head, pl.ds(c0, 128)]) + atail[:, pl.ds(c0, 128)]
            kt = r[0:24]
            vt = r[24:48].astype(BF16).astype(F32)
            row = _iota((24, 128), 0)
            for u in range(GH):
                ku = kt if u == 0 else pltpu.roll(kt, 2 * u, 0)
                ku = jnp.concatenate([ku, jnp.zeros((8, 128), F32)], axis=0).T
                if u == 0:
                    kf[pl.ds(c0, 128), :] = ku
                ka[u, pl.ds(c0 // 2, 64), :] = _pack(ku)
                vu = vt if u == 0 else pltpu.roll(vt, 2 * u, 0)
                va[u, :, pl.ds(c0, 128)] = jnp.where((row >= 2 * u) & (row < 2 * u + DH), vu, 1.0)
            qa[:, pl.ds(c0, 128)] = r[48:] * QSCALE

    def b_project(p, c):
        zero = jnp.zeros((GP - GR, 128), F32)
        for part in (1, 0, 2):
            tiles = project(wbt, pl.multiple_of(part * (D // 2) + p * GR, 8), 2 * GR,
                            lambda k0, k, t: xb[k0:k0 + k, _tile(c * NT + t)], part, pause=True)
            yield next(tiles)
            for t, r in enumerate(tiles):
                i = c * NT + t
                if part == 2:
                    v, row = r.astype(BF16).astype(F32), _iota((8, 128), 0)
                    for y in range(2 * GH):
                        h, r0 = y % GH, (y // GH) * GR + 16 * (y % GH)
                        if h == 0:
                            win = [v[r0:r0 + 16], jnp.where(row >= 2, 1.0, v[r0 + 16:r0 + 24])]
                        else:
                            win = [jnp.where(row >= 2 * h, v[r0:r0 + 8], 1.0), v[r0 + 8:r0 + 24]]
                        vb[y, :, _tile(i)] = jnp.concatenate(win, axis=0)
                else:
                    for y in range(2):
                        rg = jnp.concatenate([r[y * GR:(y + 1) * GR], zero], axis=0)
                        if part == 0:
                            qb[y, :, _tile(i)] = _pack(rg * QSCALE)
                        else:
                            kb[y, pl.ds(pl.multiple_of(i * 64, 64), 64), :] = pltpu.bitcast(rg.astype(BF16).T, U32)
                yield

    def b_scores(y, i, after):
        q = qb[y, :, _tile(i)]
        q = jnp.concatenate([after(q[8 * r:8 * r + 8]) for r in range(GP // 16)], axis=0)
        e0 = (i % 2) * (BR // 2)
        first = max(0, 8 - 4 * i)
        keys = lambda r, m: kb[y, pl.ds(64 * (i - 2) + r, m), :]
        mid = max(first, GH - 1)
        for t in range(GH):
            band = after(msk[pl.ds(M_KEY + 8 * t, 8), :].astype(jnp.int32))[:, 0:GP]
            ks = [keys(9 * n + 8 * x, 8) if first else
                  jnp.where(band > x // 2, keys(9 * n + 8 * x, 8), keys(8 * x, 8)) for x in range(2 * (GH - 1))]
            ks.append(keys(mid * n, (9 - mid) * n))
            s = _mm(_bf16(jnp.concatenate(ks, axis=0)),
                    _bf16(q & msk[pl.ds(M_QUERY + t * (GP // 2), GP // 2), :]))
            if first:
                eb[e0:e0 + 3 * n, _tile(t)] = _pack(jnp.exp2(s[0:3 * BAND]))
                eb[e0 + mid * n:e0 + 9 * n, _tile(t)] = _pack(jnp.exp2(s[3 * BAND:]))
            else:
                eb[e0:e0 + 9 * n, _tile(t)] = _pack(jnp.exp2(s))
        return s

    def b_unskew(i, x, after):
        e0 = (i % 2) * (BR // 2)
        band = after(_iota((8, 128), 1) >> 5)
        band = jnp.concatenate([band, band], axis=0)
        odd_band, high_band = (band & 1) == 1, band >= 2
        out = [[] for _ in range(GH)]
        for blk in range(4 * x, 4 * x + 4):
            src = [eb[pl.ds(e0 + (blk % 9) * n, n), _tile(t)] for t in range(GH)]
            if blk == 0:
                res = src
            elif blk == 11:
                res = [src[(h - 3) % GH] for h in range(GH)]
            else:
                res = [jnp.where(odd_band, src[(h - 1) % GH], src[h]) for h in range(GH)]
                if blk == 10:
                    res = [res[(h - 2) % GH] for h in range(GH)]
                elif blk > 1:
                    res = [jnp.where(high_band, res[(h - 2) % GH], res[h]) for h in range(GH)]
            if x != 1:
                mask = msk[pl.ds(M_OLD + n * blk if x == 0 else M_NEW + n * (blk - 8), n), :]
                res = [r & mask for r in res]
            for h in range(GH):
                out[h].append(res[h])
        return [_bf16(jnp.concatenate(o, axis=0)) for o in out]

    def b_store(p, y, i, outs):
        ob[pl.ds(pl.multiple_of((2 * p + y) * GR, 8), GR), _tile(i)] = _stitch(outs)

    def b_output(p, y, i, z, pause=lambda: None, after=lambda x: lambda v: v):
        outs = [None] * GH
        for x in range(3):
            if i + x >= 2:
                for h, e in enumerate(b_unskew(i, x, after(x))):
                    a = _mm(vb[y * GH + h, :, _tile(i + x - 2)], e)
                    outs[h] = a if outs[h] is None else outs[h] + a
            pause()
        for h in range(GH):
            outs[h], z = _normalise(outs[h], h, z)
        b_store(p, y, i, outs)
        return z

    def b_step(p, z):
        w = p % 2
        wot[pl.ds(pl.multiple_of(w * (D // 2), 8), D // 2), :] = pltpu.bitcast(wo[w].T, U32)
        always = _always(p)

        def after(dep, row):
            if dep is None:
                return lambda v: v
            row = min(row, dep.shape[0] - 8)
            return lambda v: jnp.where(always, v, pltpu.bitcast(dep[row:row + 8], v.dtype))

        proj, s, prev = b_project(p, 0), None, None
        z = b_output(jnp.maximum(p - 1, 0), 1, NB * NT - 1, z, lambda: next(proj))
        for c in range(NB):
            for _ in proj:
                pass
            proj = b_project(p, c + 1) if c + 1 < NB else iter(())
            rows = (0, 160, 280, 280) if c + 1 < NB else (0, 40, 80, 160)
            for y in range(2):
                for i in range(c * NT, (c + 1) * NT):
                    s = b_scores(y, i, after(s, rows[3]))
                    pauses = iter([True, True, False])
                    pause = lambda: next(pauses) and next(proj, None)
                    if prev:
                        z = b_output(p, *prev, z, pause, lambda x: after(s, rows[x]))
                    else:
                        pause()
                    prev = (y, i)
        return z

    def a_stage(j, u):
        qs[u] = qa[pl.ds(pl.multiple_of((j % NG) * GR + 16 * u, 8), 24),
                   pl.ds(pl.multiple_of((j // NG) * QB, QB), QB)]

    def a_query(u):
        return jnp.concatenate([qs[u], jnp.zeros((8, QB), F32)], axis=0).astype(BF16)

    def a_store(j, u, acc):
        oa[(j % NG) * GH + u, :, pl.ds(pl.multiple_of((j // NG) * QB, QB), QB)] = acc

    def a_output(j, u):
        acc = None
        for c in range(NC):
            p = pa[pl.ds(((u % 2) * S + c * KC) // 2, KC // 2), :]
            a = _mm(va[u, :, _tile(c)], _bf16(p))
            acc = a if acc is None else acc + a
            if c == NC - 1:
                a_store(j, u, acc)
            yield

    def a_step(step, _):
        vpu = _VpuScores(step)
        for j, u in [(step * A_UNROLL + y, u) for y in range(A_UNROLL) for u in range(GH)]:
            pv = a_output(jnp.maximum(j - 1, 0), GH - 1) if u == 0 else a_output(j, u - 1)
            p0, q, slot = (u % 2) * (S // 2), a_query(u), 0
            for c in range(NC):
                next(pv)
                m = (KC - 16 * SLOTS[c]) // 2
                s = _mm(_bf16(ka[u, pl.ds(c * (KC // 2), m), :]), q)
                pa[pl.ds(p0 + c * (KC // 2), m), :] = _pack(jnp.exp2(s))
                while slot < NS and slot * NC < (c + 1) * NS:
                    for t in range(NT):
                        vpu(lambda d: ktab[slot, pl.ds(16 * d, 16), :],
                            lambda d: qs[u, pl.ds(2 * u + d, 1), t * 128:(t + 1) * 128],
                            pa.at[pl.ds(p0 + SLOT_KEY[slot] // 2, 8), t * 128:(t + 1) * 128])
                    slot += 1
            a_stage(jnp.minimum(j + 1, NB * NG - 1), u)
        return 0

    for u in range(GH):
        a_stage(0, u)
    lax.fori_loop(0, NB * NG // A_UNROLL, a_step, 0)
    for cp in late_copies:
        cp.wait()
    z = lax.fori_loop(0, NG // 2, b_step, jnp.zeros((8, 128), F32))
    z = b_output(NG // 2 - 1, 1, NB * NT - 1, z)
    for _ in a_output(NB * NG - 1, GH - 1):
        pass

    def attend_exact():
        def a_exact(step, _):
            j, u = step // GH, step % GH
            a_stage(j, u)
            q = a_query(u)

            def scores(c):
                return _mm(_bf16(ka[u, pl.ds(pl.multiple_of(c * (S // 4), S // 4), S // 4), :]), q)

            def values(c):
                return va[u, :, pl.ds(pl.multiple_of(c * (S // 2), S // 2), S // 2)]

            m = lax.fori_loop(
                0, 2, lambda c, m: jnp.maximum(m, jnp.max(scores(c), axis=0, keepdims=True)),
                jnp.full((1, QB), -jnp.inf, F32))
            acc = lax.fori_loop(
                0, 2, lambda c, acc: acc + _mm(values(c), jnp.exp2(scores(c) - m).astype(BF16)),
                jnp.zeros((24, QB), F32))
            a_store(j, u, acc)
            return 0

        def b_exact(p, _):
            def project_block(c, _):
                for _ in b_project(p, c):
                    pass
                return 0

            def attend(step, _):
                y, i = step // (NB * NT), step % (NB * NT)
                k0 = jnp.maximum(i - 2, 0)
                q = qb[y, :, _tile(i)]
                k = _bf16(kb[y, pl.ds(pl.multiple_of(k0 * 64, 64), 192), :])
                dist = _iota((384, 128), 1) - _iota((384, 128), 0) + (i - k0) * 128
                keep = (dist >= 0) & (dist < W)
                row = _iota(q.shape, 0)
                qh = [jnp.where((row >= h * (DH // 2)) & (row < (h + 1) * (DH // 2)), q, none) for h in range(GH)]
                s4 = _mm(k, _bf16(jnp.concatenate(qh, axis=1)))
                outs = []
                for h in range(GH):
                    s = jnp.where(keep, s4[:, h * 128:(h + 1) * 128], NEG)
                    e = jnp.exp2(s - jnp.max(s, axis=0, keepdims=True)).astype(BF16)
                    v = vb[y * GH + h, :, pl.ds(pl.multiple_of(k0 * 128, 128), 384)]
                    outs.append(_normalise(_mm(v, e), h, z)[0])
                b_store(p, y, i, outs)
                return 0

            lax.fori_loop(0, NB, project_block, 0)
            lax.fori_loop(0, 2 * NB * NT, attend, 0)
            return 0

        lax.fori_loop(0, NB * H, a_exact, 0)
        lax.fori_loop(0, NG // 2, b_exact, 0)

    def out_copy(i):
        return pltpu.make_async_copy(obuf.at[_tile(i), :], out_hbm.at[_tile(i), :], out_sem.at[i])

    def proj_o(c, z):
        always, spare, started = _always(c), pl.multiple_of(S + 16 * jnp.minimum(c, 0), 16), {}

        def mark(t):
            obuf[pl.ds(spare, 16), 0:128] = jnp.zeros((16, 128), BF16)
            started[t] = pltpu.bitcast(obuf[pl.ds(spare + 16, 16), 0:128], F32)

        def b_tile(k0, k, t):
            x = ob[k0:k0 + k, _tile(c * NT + t)]
            if k0 == 0 and t in started:
                x = jnp.concatenate([jnp.where(always, x[r:r + 8], started[t]) if r % 64 == 0 else x[r:r + 8]
                                     for r in range(0, k, 8)], axis=0)
            return x.astype(BF16)

        late = jnp.maximum(c * NT - 1, 0)
        obuf[_tile(late), 0:LATE] = _bf16(ybuf[...]).T

        @pl.when(c > 0)
        def _():
            out_copy(late).start()

        mark(1)
        xs = []
        for t in range(NT):
            groups = []
            for g in range(NG):
                outs = []
                for u in range(GH):
                    o, z = _normalise(oa[g * GH + u, :, _tile(c * NT + t)], u, z)
                    outs.append(o)
                groups.append(_stitch(outs))
            xs.append(jnp.concatenate(groups, axis=0))
        yb = project(wot, D // 2, D, b_tile, 1)
        ya = project(wot, 0, D, lambda k0, k, t: xs[t][k0:k0 + k].astype(BF16), 0)
        for t, (b, a) in enumerate(zip(yb, ya)):
            y = jnp.concatenate([a, b], axis=0)
            if t < NT - 1:
                obuf[_tile(c * NT + t), :] = y.astype(BF16).T
                out_copy(c * NT + t).start()
                if t + 2 < NT:
                    mark(t + 2)
            else:
                obuf[_tile(c * NT + t), LATE:] = y[LATE:].astype(BF16).T
                ybuf[...] = _pack(y[:LATE])
        return z

    def finish(exact):
        pl.when(exact == 1)(attend_exact)
        check = lax.fori_loop(0, NB, proj_o, z)
        obuf[_tile(NB * NT - 1), 0:LATE] = _bf16(ybuf[...]).T
        out_copy(NB * NT - 1).start()
        unsafe = jnp.max(jnp.where(check < 2.0 ** 120, 0, 1))
        for i in range(NB * NT):
            out_copy(i).wait()
        return jnp.where(unsafe > 0, exact + 1, 2)

    lax.while_loop(lambda exact: exact < 2, finish, jnp.int32(0))


@jax.jit
def pallas_concat_heads__grouped_kv_mqa__sliding_block__prompt_kernel(
    A_x: jax.Array,
    A_wq: jax.Array,
    A_wk: jax.Array,
    A_wv: jax.Array,
    A_wo: jax.Array,
    B_x: jax.Array,
    B_wqkv: jax.Array,
    B_wo: jax.Array,
):
    hbm = pl.BlockSpec(memory_space=pltpu.HBM)
    vmem = pltpu.VMEM
    out = pl.pallas_call(
        _kernel,
        in_specs=[hbm] * 8,
        out_specs=hbm,
        out_shape=jax.ShapeDtypeStruct((S, 2 * D), BF16),
        scratch_shapes=[
            vmem((D, S), BF16), vmem((D, D), BF16), vmem((DH, D), BF16), vmem((DH, D), BF16),
            vmem((D, S), BF16), vmem((D, 3 * D), BF16), vmem((2, D, D), BF16),
            vmem((D // 2 + 24, D), U32), vmem((3 * D // 2, D), U32), vmem((D, D), U32),
            vmem((D + 48, S), F32), vmem((3, D, QB), F32),
            vmem((D, S), F32), vmem((GH, 24, QB), F32), vmem((GH, S // 2, 32), U32),
            vmem((S, 32), F32), vmem((GH, 24, S), F32), vmem((NS, 16 * DH + 8, 128), F32),
            vmem((S, QB), U32), vmem((H, 24, S), F32),
            vmem((2, GP // 2, S), U32), vmem((2, S // 2, GP), U32), vmem((2 * GH, 24, S), F32),
            vmem((BR, QB), U32), vmem((D, S), F32), vmem((M_ROWS, 128), U32),
            vmem((LATE // 2, 128), U32), vmem((S + 32, 2 * D), BF16),
            pltpu.SemaphoreType.DMA((9 + NB,)), pltpu.SemaphoreType.DMA((NB * NT,)),
        ],
        compiler_params=pltpu.CompilerParams(vmem_limit_bytes=100 * 1024 * 1024),
        name="mqa_swa_fused",
    )(A_x[0].T, A_wq, A_wk.T, A_wv.T, A_wo, B_x[0].T, B_wqkv, B_wo)
    return out[None]
```
